```python
import os as _os
_os.environ.setdefault("JAX_PLATFORMS", "cpu")
import jax
import jax.numpy as jnp

def _softmax(x, axis=-1):
    return jax.nn.softmax(x, axis=axis)
def _gelu(x):
    return jax.nn.gelu(x, approximate=True)
def _silu(x):
    return jax.nn.silu(x)
def _sigmoid(x):
    return jax.nn.sigmoid(x)
def _layernorm(x, axis=-1, eps=1e-5):
    m = jnp.mean(x, axis=axis, keepdims=True)
    v = jnp.var(x, axis=axis, keepdims=True)
    return (x - m) / jnp.sqrt(v + eps)
def _scatter_add(tgt, idx, src, axis=0):
    return tgt.at[idx].add(src)
def _segment_sum(src, seg, n):
    return jax.ops.segment_sum(src, seg, n)
class _Rng:
    def __init__(self, key):
        self._k = key
    def _next(self):
        self._k, sub = jax.random.split(self._k)
        return sub
    def normal(self, shape):
        return jax.random.normal(self._next(), shape, dtype=jnp.bfloat16)
    def randint(self, lo, hi, shape):
        return jax.random.randint(self._next(), shape, lo, hi, dtype=jnp.int32)
    def uniform(self, shape, lo=0.0, hi=1.0):
        return jax.random.uniform(self._next(), shape, jnp.bfloat16, lo, hi)
    def permutation(self, n):
        return jax.random.permutation(self._next(), n)


kernel_name = 'parallel_sum__mha_block__swiglu_ffn__prompt'

def setup_inputs():
    _rng = _Rng(jax.random.key(int.from_bytes(__import__("os").urandom(4), "little")))
    _w = (lambda a: (lambda t: t.astype(jnp.bfloat16) if jnp.issubdtype(t.dtype, jnp.floating) else t)(jnp.asarray(a)))
    def _A_setup():
        B, S, D, H = 1, 2048, 512, 32
        return {
            "x": _w((lambda *s: _rng.normal(s) * 0.05)(B, S, D)),
            "wqkv": _w((lambda *s: _rng.normal(s) * 0.1)(D, 3 * D)),
            "wo": _w((lambda *s: _rng.normal(s) * 0.05)(D, D)),
        }
    _A_in = _A_setup()

    def _B_setup():
        B, S, D, F = 1, 2048, 512, 1792
        return {
            "x": _w((lambda *s: _rng.normal(s) * 0.05)(B, S, D)),
            "w_gate": _w((lambda *s: _rng.normal(s) * 0.05)(D, F)),
            "w_up": _w((lambda *s: _rng.normal(s) * 0.05)(D, F)),
            "w_down": _w((lambda *s: _rng.normal(s) * 0.05)(F, D)),
        }
    _B_in = _B_setup()

    return {
        "A_x": _A_in["x"],
        "A_wqkv": _A_in["wqkv"],
        "A_wo": _A_in["wo"],
        "B_x": _B_in["x"],
        "B_w_gate": _B_in["w_gate"],
        "B_w_up": _B_in["w_up"],
        "B_w_down": _B_in["w_down"],
    }

def reference(A_x, A_wqkv, A_wo, B_x, B_w_gate, B_w_up, B_w_down):
    def _A_ref(x, wqkv, wo):
        B, S, D = x.shape
        H = 32
        Dh = D // H
        qkv = (lambda x, *d: x.transpose(*d))((x @ wqkv).reshape(B, S, 3, H, Dh), 2, 0, 3, 1, 4)
        q, k, v = qkv[0], qkv[1], qkv[2]
        scores = jnp.einsum("bhqd,bhkd->bhqk", q, k) * (Dh ** -0.5)
        p = _softmax(scores, axis=-1)
        o = jnp.einsum("bhqk,bhkd->bhqd", p, v)
        return (lambda x, *d: x.transpose(*d))(o, 0, 2, 1, 3).reshape(B, S, D) @ wo

    def _B_ref(x, w_gate, w_up, w_down):
        g = _silu(x @ w_gate)
        u = x @ w_up
        return (g * u) @ w_down

    x = A_x
    xn = _layernorm(x, axis=-1)
    return x + _A_ref(xn, A_wqkv, A_wo) + _B_ref(xn, B_w_gate, B_w_up, B_w_down)
```

```python
import math

import jax
import jax.numpy as jnp
from jax import lax
from jax.experimental import pallas as pl
from jax.experimental.pallas import tpu as pltpu

_H = 32
_TQ = 512
_TK = 128
_RB = 512
_FB = 256
_F32 = jnp.float32
_BF16 = jnp.bfloat16


def _kernel(x_hbm, wqkv_hbm, wo_hbm, wg_hbm, wu_hbm, wd_hbm, out_hbm,
            x_v, wqkv_v, wo_v, wg_v, wu_v, wd_v,
            xn_v, qt_v, k_v, vt_v, ot_v, s_v, qn_v, h_v, out_v,
            xsem, wsem, osem):
    S, D = x_v.shape
    F = wg_v.shape[1]
    dh = D // _H
    hpg = 128 // dh
    nb = S // _RB

    def x_copy(b):
        return pltpu.make_async_copy(x_hbm.at[pl.ds(b * _RB, _RB)],
                                     x_v.at[pl.ds(b * _RB, _RB)], xsem.at[b])

    w_copies = [pltpu.make_async_copy(src, dst, wsem.at[j]) for j, (src, dst) in enumerate(
        ((wqkv_hbm, wqkv_v), (wg_hbm, wg_v), (wu_hbm, wu_v), (wd_hbm, wd_v), (wo_hbm, wo_v)))]

    def out_copy(b):
        return pltpu.make_async_copy(out_v.at[pl.ds(b * _RB, _RB)],
                                     out_hbm.at[pl.ds(b * _RB, _RB)], osem.at[b])

    x_copy(0).start()
    w_copies[0].start()
    for b in range(1, nb):
        x_copy(b).start()
    for c in w_copies[1:]:
        c.start()

    qscale = float(dh ** -0.5 * math.log2(math.e))
    for b in range(nb):
        rows = slice(b * _RB, (b + 1) * _RB)
        x_copy(b).wait()
        x = x_v[rows, :].astype(_F32)
        mean = jnp.mean(x, axis=-1, keepdims=True)
        xc = x - mean
        var = jnp.mean(xc * xc, axis=-1, keepdims=True)
        xn = (xc * lax.rsqrt(var + 1e-5)).astype(_BF16)
        xn_v[rows, :] = xn
        if b == 0:
            w_copies[0].wait()
        q = jnp.dot(xn, wqkv_v[:, 0:D], preferred_element_type=_F32) * qscale
        qt = q.T.astype(_BF16)
        k = jnp.dot(xn, wqkv_v[:, D:2 * D], preferred_element_type=_F32).astype(_BF16)
        vt = jnp.dot(xn, wqkv_v[:, 2 * D:3 * D], preferred_element_type=_F32).T.astype(_BF16)
        for g in range(D // 128):
            qt_v[g, :, rows] = qt[g * 128:(g + 1) * 128, :]
            k_v[g, rows, :] = k[:, g * 128:(g + 1) * 128]
        for h in range(_H):
            vt_v[h, :, rows] = vt[h * dh:(h + 1) * dh, :]

    nq = S // _TQ
    n_items = _H * nq
    nc = S // _TK

    def masked_qt(i):
        i = jnp.minimum(i, n_items - 1)
        h = i // nq
        q = qt_v[h // hpg, :, pl.ds(pl.multiple_of((i % nq) * _TQ, _TQ), _TQ)]
        row = lax.broadcasted_iota(jnp.int32, (128, _TQ), 0)
        return jnp.where(row // dh == h % hpg, q, jnp.zeros_like(q))

    def fold(a, op):
        return op(a.reshape(_TK // 8, 8, _TQ), axis=0)

    q0 = masked_qt(0)
    m0 = None
    for c in range(nc):
        sl = slice(c * _TK, (c + 1) * _TK)
        s = jnp.dot(k_v[0, sl, :], q0, preferred_element_type=_F32)
        s_v[sl, :] = s
        m0 = fold(s, jnp.max) if m0 is None else jnp.maximum(m0, fold(s, jnp.max))
    qn_v[...] = masked_qt(1)

    def att_step(i, mx):
        h = i // nq
        g1 = jnp.minimum(i + 1, n_items - 1) // (hpg * nq)
        q1 = qn_v[...]
        m = o = l = None
        for c in range(nc):
            sl = slice(c * _TK, (c + 1) * _TK)
            p = jnp.exp2(s_v[sl, :] - mx)
            lc = fold(p, jnp.sum)
            oc = jnp.dot(vt_v[h, :, sl], p.astype(_BF16), preferred_element_type=_F32)
            s = jnp.dot(k_v[g1, sl, :], q1, preferred_element_type=_F32)
            s_v[sl, :] = s
            if c == 0:
                m, o, l = fold(s, jnp.max), oc, lc
            else:
                m, o, l = jnp.maximum(m, fold(s, jnp.max)), o + oc, l + lc
        r = o / jnp.sum(l, axis=0, keepdims=True)
        ot_v[h, :, pl.ds(pl.multiple_of((i % nq) * _TQ, _TQ), _TQ)] = r.astype(_BF16)
        qn_v[...] = masked_qt(i + 2)
        return jnp.max(m, axis=0, keepdims=True)

    lax.fori_loop(0, n_items, att_step, jnp.max(m0, axis=0, keepdims=True))

    for c in w_copies[1:]:
        c.wait()

    def out_step(b, carry):
        rows = pl.ds(pl.multiple_of(b * _RB, _RB), _RB)
        xn = xn_v[rows, :]
        for f in range(F // _FB):
            cols = slice(f * _FB, (f + 1) * _FB)
            g = jnp.dot(xn, wg_v[:, cols], preferred_element_type=_F32)
            u = jnp.dot(xn, wu_v[:, cols], preferred_element_type=_F32)
            h_v[:, cols] = (g * jax.nn.sigmoid(g) * u).astype(_BF16)
        ot = ot_v[:, :, rows].reshape(D, _RB)
        y = lax.dot_general(ot, wo_v[...], (((0,), (0,)), ((), ())), preferred_element_type=_F32)
        y = y + jnp.dot(h_v[...], wd_v[...], preferred_element_type=_F32)
        out_v[rows, :] = (x_v[rows, :].astype(_F32) + y).astype(out_v.dtype)
        out_copy(b).start()
        return carry

    lax.fori_loop(0, nb, out_step, 0)
    for b in range(nb):
        out_copy(b).wait()


@jax.jit
def pallas_parallel_sum__mha_block__swiglu_ffn__prompt_kernel(
    A_x: jax.Array,
    A_wqkv: jax.Array,
    A_wo: jax.Array,
    B_x: jax.Array,
    B_w_gate: jax.Array,
    B_w_up: jax.Array,
    B_w_down: jax.Array,
):
    del B_x
    B, S, D = A_x.shape
    F = B_w_gate.shape[1]
    assert B == 1 and S % _TQ == 0 and S % _RB == 0 and F % _FB == 0 and D % 128 == 0
    dh = D // _H
    nb = S // _RB
    any_spec = pl.BlockSpec(memory_space=pl.ANY)
    out = pl.pallas_call(
        _kernel,
        out_shape=jax.ShapeDtypeStruct((S, D), A_x.dtype),
        in_specs=[any_spec] * 6,
        out_specs=any_spec,
        scratch_shapes=[
            pltpu.VMEM((S, D), A_x.dtype),
            pltpu.VMEM((D, 3 * D), A_wqkv.dtype),
            pltpu.VMEM((D, D), A_wo.dtype),
            pltpu.VMEM((D, F), B_w_gate.dtype),
            pltpu.VMEM((D, F), B_w_up.dtype),
            pltpu.VMEM((F, D), B_w_down.dtype),
            pltpu.VMEM((S, D), _BF16),
            pltpu.VMEM((D // 128, 128, S), _BF16),
            pltpu.VMEM((D // 128, S, 128), _BF16),
            pltpu.VMEM((_H, dh, S), _BF16),
            pltpu.VMEM((_H, dh, S), _BF16),
            pltpu.VMEM((S, _TQ), _F32),
            pltpu.VMEM((128, _TQ), _BF16),
            pltpu.VMEM((_RB, F), _BF16),
            pltpu.VMEM((S, D), A_x.dtype),
            pltpu.SemaphoreType.DMA((nb,)),
            pltpu.SemaphoreType.DMA((5,)),
            pltpu.SemaphoreType.DMA((nb,)),
        ],
        compiler_params=pltpu.CompilerParams(vmem_limit_bytes=100 * 1024 * 1024),
    )(A_x.reshape(S, D), A_wqkv, A_wo, B_w_gate, B_w_up, B_w_down)
    return out.reshape(B, S, D)
```

```python
import math

import jax
import jax.numpy as jnp
from jax import lax
from jax.experimental import pallas as pl
from jax.experimental.pallas import tpu as pltpu

_H = 32
_TQ = 512
_TK = 128
_RB = 512
_LNB = 128
_FB = 128
_F32 = jnp.float32
_BF16 = jnp.bfloat16


def _kernel(x_hbm, wqkv_hbm, wo_hbm, wg_hbm, wu_hbm, wd_hbm, out_hbm,
            x_v, wqkv_v, wo_v, wg_v, wu_v, wd_v,
            xn_v, qt_v, k_v, vt_v, ot_v, s_v, acc_v, h_v, out_v,
            xsem, wsem, osem):
    S, D = x_v.shape
    F = wg_v.shape[1]
    dh = D // _H
    hpg = 128 // dh
    nb = S // _RB

    def x_copy(b):
        return pltpu.make_async_copy(x_hbm.at[pl.ds(b * _RB, _RB)],
                                     x_v.at[pl.ds(b * _RB, _RB)], xsem.at[b])

    w_pairs = [(wqkv_hbm.at[:, pl.ds(j * D, D)], wqkv_v.at[j]) for j in range(3)]
    w_pairs += [(wg_hbm, wg_v), (wu_hbm, wu_v), (wo_hbm, wo_v), (wd_hbm, wd_v)]
    w_copies = [pltpu.make_async_copy(src, dst, wsem.at[j]) for j, (src, dst) in enumerate(w_pairs)]

    def out_copy(b):
        return pltpu.make_async_copy(out_v.at[pl.ds(b * _RB, _RB)],
                                     out_hbm.at[pl.ds(b * _RB, _RB)], osem.at[b])

    x_copy(0).start()
    w_copies[0].start()

    qscale = float(dh ** -0.5 * math.log2(math.e))

    def layernorm(b, part):
        r0 = b * _RB + part * _LNB
        rows = slice(r0, r0 + _LNB)
        x = x_v[rows, :].astype(_F32)
        mean = jnp.mean(x, axis=-1, keepdims=True)
        xc = x - mean
        var = jnp.mean(xc * xc, axis=-1, keepdims=True)
        xn_v[rows, :] = (xc * lax.rsqrt(var + 1e-5)).astype(_BF16)

    w_copies[1].start()
    x_copy(1).start()
    w_copies[2].start()
    for h in range(_H):
        j = h % hpg
        if j > 0:
            qt_v[h, :j * dh, :] = jnp.zeros((j * dh, S), _BF16)
        if j < hpg - 1:
            qt_v[h, (j + 1) * dh:, :] = jnp.zeros((128 - (j + 1) * dh, S), _BF16)
    x_copy(0).wait()
    for part in range(_RB // _LNB):
        layernorm(0, part)
    for b in range(nb):
        rows = slice(b * _RB, (b + 1) * _RB)
        xn = xn_v[rows, :]

        def ln_next(part):
            if b + 1 < nb:
                layernorm(b + 1, part)

        def proj(j):
            if b == 0:
                w_copies[j].wait()
            return jnp.dot(xn, wqkv_v[j], preferred_element_type=_F32)

        qt = (proj(0) * qscale).T.astype(_BF16)
        if b + 1 < nb:
            x_copy(b + 1).wait()
        halves = []
        for half in range(2):
            hr = slice(half * (_RB // 2), (half + 1) * (_RB // 2))
            if b == 0 and half == 0:
                w_copies[1].wait()
                w_copies[2].wait()
                for bb in range(2, nb):
                    x_copy(bb).start()
            kh = jnp.dot(xn[hr], wqkv_v[1], preferred_element_type=_F32).astype(_BF16)
            ln_next(2 * half)
            vh = jnp.dot(xn[hr], wqkv_v[2], preferred_element_type=_F32).T.astype(_BF16)
            ln_next(2 * half + 1)
            halves.append((kh, vh))
        k = jnp.concatenate([kv[0] for kv in halves], axis=0)
        vt = jnp.concatenate([kv[1] for kv in halves], axis=1)
        for g in range(D // 128):
            k_v[g, rows, :] = k[:, g * 128:(g + 1) * 128]
        for h in range(_H):
            j = h % hpg
            qt_v[h, j * dh:(j + 1) * dh, rows] = qt[h * dh:(h + 1) * dh, :]
            vt_v[h, :, rows] = vt[h * dh:(h + 1) * dh, :]

    for c in w_copies[3:]:
        c.start()

    nc = S // _TK
    tiles = [slice(j * _TQ, (j + 1) * _TQ) for j in range(S // _TQ)]
    chunks = [slice(c * _TK, (c + 1) * _TK) for c in range(nc)]

    def fold(a, op):
        return op(a.reshape(_TK // 8, 8, _TQ), axis=0)

    def sweep(h, mx, do_pv, do_qk, between=None):
        if do_qk:
            g1 = (h + 1) // hpg
            q1 = [qt_v[h + 1, :, t] for t in tiles]
        m = [None] * len(tiles)
        for c, sl in enumerate(chunks):
            for j, t in enumerate(tiles):
                if do_pv:
                    p = jnp.exp2(s_v[sl, t] - mx[j])
                    l = fold(p, jnp.sum)
                    o = jnp.dot(vt_v[h, :, sl], p.astype(_BF16), preferred_element_type=_F32)
                if do_qk:
                    s = jnp.dot(k_v[g1, sl, :], q1[j], preferred_element_type=_F32)
                    s_v[sl, t] = s
                    m[j] = fold(s, jnp.max)
                    if c > 0:
                        m[j] = jnp.maximum(acc_v[0:8, t], m[j])
                    if c < nc - 1:
                        acc_v[0:8, t] = m[j]
                if do_pv:
                    if c > 0:
                        l = acc_v[8:16, t] + l
                        o = acc_v[16:, t] + o
                    if c < nc - 1:
                        acc_v[8:16, t] = l
                        acc_v[16:, t] = o
                    else:
                        ot_v[h, :, t] = (o / jnp.sum(l, axis=0, keepdims=True)).astype(_BF16)
                if between is not None and j % 2 == 1:
                    between()
        if do_qk:
            return tuple(jnp.max(v, axis=0, keepdims=True) for v in m)

    mx = sweep(-1, None, False, True)
    mx = lax.fori_loop(0, _H - 1, lambda h, mx: sweep(h, mx, True, True), mx)

    for c in w_copies[3:]:
        c.wait()

    def ffn_hidden(rows):
        xn = xn_v[rows, :]
        for f in range(F // _FB):
            cols = slice(f * _FB, (f + 1) * _FB)
            g = jnp.dot(xn, wg_v[:, cols], preferred_element_type=_F32)
            yield
            u = jnp.dot(xn, wu_v[:, cols], preferred_element_type=_F32)
            h_v[:, cols] = (g * jax.nn.sigmoid(g) * u).astype(_BF16)
            yield

    def project_out(b, rows):
        ot = ot_v[:, :, rows].reshape(D, _RB)
        y = lax.dot_general(ot, wo_v[...], (((0,), (0,)), ((), ())), preferred_element_type=_F32)
        y = y + jnp.dot(h_v[...], wd_v[...], preferred_element_type=_F32)
        out_v[rows, :] = (x_v[rows, :].astype(_F32) + y).astype(out_v.dtype)
        out_copy(b).start()

    def out_step(b, carry):
        rows = pl.ds(pl.multiple_of(b * _RB, _RB), _RB)
        for _ in ffn_hidden(rows):
            pass
        project_out(b, rows)
        return carry

    first = ffn_hidden(slice(0, _RB))
    next(first)
    sweep(_H - 1, mx, True, False, between=lambda: next(first, None))
    for _ in first:
        pass
    project_out(0, slice(0, _RB))
    lax.fori_loop(1, nb, out_step, 0)
    for b in range(nb):
        out_copy(b).wait()


@jax.jit
def pallas_parallel_sum__mha_block__swiglu_ffn__prompt_kernel(
    A_x: jax.Array,
    A_wqkv: jax.Array,
    A_wo: jax.Array,
    B_x: jax.Array,
    B_w_gate: jax.Array,
    B_w_up: jax.Array,
    B_w_down: jax.Array,
):
    del B_x
    B, S, D = A_x.shape
    F = B_w_gate.shape[1]
    assert B == 1 and S % _TQ == 0 and S % _RB == 0 and F % _FB == 0 and D % 128 == 0
    dh = D // _H
    nb = S // _RB
    any_spec = pl.BlockSpec(memory_space=pl.ANY)
    out = pl.pallas_call(
        _kernel,
        out_shape=jax.ShapeDtypeStruct((S, D), A_x.dtype),
        in_specs=[any_spec] * 6,
        out_specs=any_spec,
        scratch_shapes=[
            pltpu.VMEM((S, D), A_x.dtype),
            pltpu.VMEM((3, D, D), A_wqkv.dtype),
            pltpu.VMEM((D, D), A_wo.dtype),
            pltpu.VMEM((D, F), B_w_gate.dtype),
            pltpu.VMEM((D, F), B_w_up.dtype),
            pltpu.VMEM((F, D), B_w_down.dtype),
            pltpu.VMEM((S, D), _BF16),
            pltpu.VMEM((_H, 128, S), _BF16),
            pltpu.VMEM((D // 128, S, 128), _BF16),
            pltpu.VMEM((_H, dh, S), _BF16),
            pltpu.VMEM((_H, dh, S), _BF16),
            pltpu.VMEM((S, S), _F32),
            pltpu.VMEM((16 + dh, S), _F32),
            pltpu.VMEM((_RB, F), _BF16),
            pltpu.VMEM((S, D), A_x.dtype),
            pltpu.SemaphoreType.DMA((nb,)),
            pltpu.SemaphoreType.DMA((7,)),
            pltpu.SemaphoreType.DMA((nb,)),
        ],
        compiler_params=pltpu.CompilerParams(vmem_limit_bytes=100 * 1024 * 1024),
    )(A_x.reshape(S, D), A_wqkv, A_wo, B_w_gate, B_w_up, B_w_down)
    return out.reshape(B, S, D)
```
